```python
import os as _os
_os.environ.setdefault("JAX_PLATFORMS", "cpu")
import jax
import jax.numpy as jnp

def _softmax(x, axis=-1):
    return jax.nn.softmax(x, axis=axis)
def _gelu(x):
    return jax.nn.gelu(x, approximate=True)
def _silu(x):
    return jax.nn.silu(x)
def _sigmoid(x):
    return jax.nn.sigmoid(x)
def _layernorm(x, axis=-1, eps=1e-5):
    m = jnp.mean(x, axis=axis, keepdims=True)
    v = jnp.var(x, axis=axis, keepdims=True)
    return (x - m) / jnp.sqrt(v + eps)
def _scatter_add(tgt, idx, src, axis=0):
    return tgt.at[idx].add(src)
def _segment_sum(src, seg, n):
    return jax.ops.segment_sum(src, seg, n)
class _Rng:
    def __init__(self, key):
        self._k = key
    def _next(self):
        self._k, sub = jax.random.split(self._k)
        return sub
    def normal(self, shape):
        return jax.random.normal(self._next(), shape, dtype=jnp.bfloat16)
    def randint(self, lo, hi, shape):
        return jax.random.randint(self._next(), shape, lo, hi, dtype=jnp.int32)
    def uniform(self, shape, lo=0.0, hi=1.0):
        return jax.random.uniform(self._next(), shape, jnp.bfloat16, lo, hi)
    def permutation(self, n):
        return jax.random.permutation(self._next(), n)


kernel_name = 'parallel_sum__spectral_gfnet__glu_gated_swiglu__prompt'

def setup_inputs():
    _rng = _Rng(jax.random.key(int.from_bytes(__import__("os").urandom(4), "little")))
    _w = (lambda a: (lambda t: t.astype(jnp.bfloat16) if jnp.issubdtype(t.dtype, jnp.floating) else t)(jnp.asarray(a)))
    def _A_setup():
        B, S, D = 1, 2048, 512
        Df = D // 2 + 1
        return {
            "x": _w((lambda *s: _rng.normal(s) * 0.05)(B, S, D)),
            "w_r": _w((lambda *s: _rng.normal(s) * 0.2)(S, Df) * 0.02),
            "w_i": _w((lambda *s: _rng.normal(s) * 0.2)(S, Df) * 0.02),
        }
    _A_in = _A_setup()

    def _B_setup():
        B, S, D, F = 1, 2048, 512, 1376
        return {
            "x": _w((lambda *s: _rng.normal(s) * 0.05)(B, S, D)),
            "w1": _w((lambda *s: _rng.normal(s) * 0.05)(D, F) * (2.0 / D) ** 0.5),
            "w3": _w((lambda *s: _rng.normal(s) * 0.05)(D, F) * (2.0 / D) ** 0.5),
            "w2": _w((lambda *s: _rng.normal(s) * 0.05)(F, D) * (2.0 / F) ** 0.5),
        }
    _B_in = _B_setup()

    return {
        "A_x": _A_in["x"],
        "A_w_r": _A_in["w_r"],
        "A_w_i": _A_in["w_i"],
        "B_x": _B_in["x"],
        "B_w1": _B_in["w1"],
        "B_w3": _B_in["w3"],
        "B_w2": _B_in["w2"],
    }

def reference(A_x, A_w_r, A_w_i, B_x, B_w1, B_w3, B_w2):
    def _A_ref(x, w_r, w_i):
        B, S, D = x.shape
        X = (lambda x, axes=(-2,-1): jnp.fft.rfft2(x.astype(jnp.float32), axes=axes))(x, axes=(-2, -1))
        W = w_r + 1j * w_i
        X = X * W
        y = (lambda x, s, axes=(-2,-1): jnp.fft.irfft2(x, s=s, axes=axes).astype(jnp.bfloat16))(X, (S, D), axes=(-2, -1))
        return y

    def _B_ref(x, w1, w3, w2):
        gate = jnp.einsum("bsd,df->bsf", x, w1)
        up = jnp.einsum("bsd,df->bsf", x, w3)
        h = _silu(gate) * up
        out = jnp.einsum("bsf,fd->bsd", h, w2)
        return out

    x = A_x
    xn = _layernorm(x, axis=-1)
    return x + _A_ref(xn, A_w_r, A_w_i) + _B_ref(xn, B_w1, B_w3, B_w2)
```

```python
import numpy as np
import jax
import jax.numpy as jnp
from jax import lax
import jax.experimental.pallas as pl
import jax.experimental.pallas.tpu as pltpu

S, D, F = 2048, 512, 1376
R = 272
BF = jnp.bfloat16
F32 = jnp.float32
F0 = 384
NT = (((1,), (1,)), ((), ()))


def _consts():
    n = np.arange(256)[None, :]
    j = np.arange(128)[:, None]
    te = 2 * np.pi * n * j / 256
    to = 2 * np.pi * n * (2 * j + 1) / 512
    ny = np.zeros((16, 256))
    ny[0] = (-1.0) ** np.arange(256)
    fd = np.concatenate([np.cos(te), -np.sin(te), ny, np.cos(to), -np.sin(to)], 0)
    ge = np.concatenate([2 * np.cos(te), -2 * np.sin(te)], 0)
    ge[0] = 1.0
    ge[128] = ny[0]
    go = np.concatenate([2 * np.cos(to), -2 * np.sin(to)], 0)
    g = np.concatenate([ge, go], 0) / 512
    b = np.arange(128)[:, None]
    kb = np.arange(128)[None, :]
    mf, mi = [], []
    for a in range(16):
        t = 2 * np.pi * (16 * b + a) * kb / 2048
        c, s = np.cos(t), np.sin(t)
        mf.append(np.block([[c, -s], [s, c]]))
        mi.append(np.block([[c, -s], [s, c]]) / 2048)
    f = lambda v: np.asarray(v, np.float32).astype(BF)
    return f(fd), f(g), f(np.stack(mf))


_FD, _G, _MF = _consts()
_H = np.float32(np.sqrt(0.5))
_C8, _S8 = np.float32(np.cos(np.pi / 8)), np.float32(np.sin(np.pi / 8))


def _fft4(v, sg):
    (ar, ai), (br, bi), (cr, ci), (dr, di) = v
    pr, pi, mr, mi = ar + cr, ai + ci, ar - cr, ai - ci
    qr, qi, nr, ni = br + dr, bi + di, br - dr, bi - di
    o1, o3 = (mr + ni, mi - nr), (mr - ni, mi + nr)
    if sg > 0:
        o1, o3 = o3, o1
    return [(pr + qr, pi + qi), o1, (pr - qr, pi - qi), o3]


def _rot(v, e, sg):
    r, i = v
    if e == 0:
        return v
    if e == 4:
        return (-i, r) if sg > 0 else (i, -r)
    if e == 2:
        return ((r - i) * _H, (r + i) * _H) if sg > 0 else ((r + i) * _H, (i - r) * _H)
    if e == 6:
        return ((-r - i) * _H, (r - i) * _H) if sg > 0 else ((i - r) * _H, (-r - i) * _H)
    c, s = {1: (_C8, _S8), 3: (_S8, _C8), 9: (-_C8, -_S8)}[e]
    s = s * np.float32(sg)
    return (r * c - i * s, r * s + i * c)


def _fft16(v, sg):
    st = [_fft4([v[q], v[q + 4], v[q + 8], v[q + 12]], sg) for q in range(4)]
    out = [None] * 16
    for k in range(4):
        o = _fft4([_rot(st[q][k], q * k, sg) for q in range(4)], sg)
        for l in range(4):
            out[k + 4 * l] = o[l]
    return out


def _unpack(w):
    lo = lax.bitcast_convert_type(w << 16, F32)
    hi = lax.bitcast_convert_type(w & np.int32(-65536), F32)
    return lo, hi


def _kernel(x_h, wr_h, wi_h, w1_h, w3_h, w2_h, fd_h, g_h, mf_h, o_h,
            xb, ob, wr, wi, w1, w3, w2, fd, g, mf, xn, t, v, v0, h, pq, si, so):
    xi = x_h.bitcast(jnp.int32)
    oi = o_h.bitcast(jnp.int32)
    cp = pltpu.make_async_copy
    cx = [cp(xi.at[:, m, :], xb.at[m], si.at[m]) for m in range(8)]
    lo, hi = pl.ds(0, F0), pl.ds(F0, F - F0)
    c_w1a, c_w3a, c_fd, c_mf, c_w1, c_w3, c_wr, c_wi, c_w2, c_g = [
        cp(a, b, si.at[8 + i]) for i, (a, b) in enumerate(
            [(w1_h.at[lo], w1.at[lo]), (w3_h.at[lo], w3.at[lo]), (fd_h, fd), (mf_h, mf),
             (w1_h.at[hi], w1.at[hi]), (w3_h.at[hi], w3.at[hi]),
             (wr_h, wr), (wi_h, wi), (w2_h, w2), (g_h, g)])]
    issue = [[c_fd], [cx[3], cx[4], c_mf], [], [cx[5], cx[6], c_w1], [c_w3],
             [cx[7], c_wr], [c_wi], [c_w2, c_g]]

    def ln(m):
        x = jnp.concatenate(_unpack(xb[m]), 0)
        xc = x - jnp.mean(x, -1, keepdims=True)
        y = xc * lax.rsqrt(jnp.mean(xc * xc, -1, keepdims=True) + 1e-5)
        xn[m] = y.astype(BF)
        pq[m, 0] = (y[:, :256] + y[:, 256:]).astype(BF)
        pq[m, 1] = (y[:, :256] - y[:, 256:]).astype(BF)

    def fwd(m):
        p, q = pq[m, 0], pq[m, 1]
        e = lax.dot_general(fd[:R], p, NT, preferred_element_type=F32).astype(BF)
        o = lax.dot_general(fd[R:], q, NT, preferred_element_type=F32).astype(BF)
        for u in range(2):
            c = slice(128 * u, 128 * u + 128)
            re = jnp.concatenate([e[:128, c], o[:128, c], e[256:, c]], 0)
            im = jnp.concatenate([e[128:256, c], o[128:, c], jnp.zeros((16, 128), BF)], 0)
            t[2 * m + u] = jnp.dot(jnp.concatenate([re, im], 1), mf[2 * m + u],
                                   preferred_element_type=F32)

    def up(m, f):
        y = xn[m]
        a = lax.dot_general(y, w1[f], NT, preferred_element_type=F32)
        b = lax.dot_general(y, w3[f], NT, preferred_element_type=F32)
        hf = a * 0.5
        h[m, :, f] = ((hf * jnp.tanh(hf) + hf) * b).astype(BF)
        return a

    def spec(r0, wre, wim, dep=None, keep=None):
        z = [(t[a, pl.ds(r0, 16), :128], t[a, pl.ds(r0, 16), 128:]) for a in range(16)]
        if dep is not None:
            z = [tuple(jnp.where(keep, c, dep[16 * a:16 * a + 16, :128]) for c in z[a])
                 for a in range(16)]
        z = _fft16(z, -1)
        for k in range(16):
            a, b = wre[:, 128 * k:128 * k + 128], wim[:, 128 * k:128 * k + 128]
            z[k] = (z[k][0] * a - z[k][1] * b, z[k][0] * b + z[k][1] * a)
        return _fft16(z, 1)

    def mid(i):
        a0, a1 = _unpack(pltpu.bitcast(wr[pl.ds(pl.multiple_of(32 * i, 32), 32)], jnp.int32))
        b0, b1 = _unpack(pltpu.bitcast(wi[pl.ds(pl.multiple_of(32 * i, 32), 32)], jnp.int32))
        for r0, wre, wim, f in ((16 * i, a0, b0, slice(F0, 896)),
                                (128 + 16 * i, a1, b1, slice(896, F))):
            dep = up(i, f)
            r0 = pl.multiple_of(r0, 16)
            z = spec(r0, wre, wim, dep, lax.broadcasted_iota(jnp.int32, (16, 128), 0) + i >= 0)
            for a in range(16):
                v[a, pl.ds(r0, 16), :] = jnp.concatenate(z[a], 1).astype(BF)

    def nyq():
        z = spec(256, wr[256:257].astype(F32), wi[256:257].astype(F32))
        first = lax.broadcasted_iota(jnp.int32, (16, 256), 0) == 0
        for a in range(16):
            n = jnp.concatenate([-z[a][1], z[a][0]], 1)
            v0[a] = jnp.where(first, n, v[a, :16, :].astype(F32)).astype(BF)

    def down(m):
        ye, yo = [], []
        for a in (2 * m, 2 * m + 1):
            er = lax.dot_general(mf[a, :128], v[a, :128], NT, preferred_element_type=F32)
            ve = jnp.concatenate([v0[a], v[a, 16:128]], 0)
            ei = lax.dot_general(mf[a, 128:], ve, NT, preferred_element_type=F32)
            oo = lax.dot_general(mf[a], v[a, 128:], NT, preferred_element_type=F32)
            ye.append(jnp.concatenate([er, ei], 1).astype(BF))
            yo.append(jnp.concatenate([oo[:128], oo[128:]], 1).astype(BF))
        e = jnp.dot(jnp.concatenate(ye, 0), g[:256], preferred_element_type=F32)
        o = jnp.dot(jnp.concatenate(yo, 0), g[256:], preferred_element_type=F32)
        f = jnp.dot(h[m], w2[...], preferred_element_type=F32)
        y = (jnp.concatenate(_unpack(xb[m]), 0) + f
             + jnp.concatenate([e + o, e - o], 1) * np.float32(1.0 / S))
        bits = lax.bitcast_convert_type(y.astype(BF).astype(F32), jnp.int32)
        ob[m] = lax.shift_right_logical(bits[:128], 16) | bits[128:]
        for n in {2: (0, 1, 2), 6: (3, 4, 5, 6), 7: (7,)}.get(m, ()):
            cp(ob.at[n], oi.at[:, n, :], so.at[n]).start()

    for c in (cx[0], c_w1a, c_w3a, cx[1], cx[2]):
        c.start()
    cx[0].wait()
    ln(0)
    c_w1a.wait()
    c_w3a.wait()
    for m in range(8):
        if m % 2 == 0:
            for c in issue[m] + issue[m + 1]:
                c.start()
            for c in cx[m + 1:m + 3]:
                c.wait()
        if m < 7:
            ln(m + 1)
        up(m, lo)
    c_fd.wait()
    c_mf.wait()
    for m in range(8):
        fwd(m)
    for c in (c_w1, c_w3, c_wr, c_wi):
        c.wait()

    @pl.loop(0, 8, unroll=4)
    def _(i):
        mid(i)

    c_w2.wait()
    c_g.wait()
    nyq()
    for m in range(8):
        down(m)
    for m in range(8):
        cp(ob.at[m], oi.at[:, m, :], so.at[m]).wait()


@jax.jit
def pallas_parallel_sum__spectral_gfnet__glu_gated_swiglu__prompt_kernel(
        A_x, A_w_r, A_w_i, B_x, B_w1, B_w3, B_w2):
    del B_x
    V = pltpu.VMEM
    out = pl.pallas_call(
        _kernel,
        out_shape=jax.ShapeDtypeStruct((S // 16, 16, D), BF),
        in_specs=[pl.BlockSpec(memory_space=pl.ANY)] * 9,
        out_specs=pl.BlockSpec(memory_space=pl.ANY),
        scratch_shapes=[
            V((8, 128, D), jnp.int32), V((8, 128, D), jnp.int32),
            V((257, S), BF), V((257, S), BF), V((F, D), BF), V((F, D), BF), V((F, D), BF),
            V(_FD.shape, BF), V(_G.shape, BF), V(_MF.shape, BF),
            V((8, 256, D), BF), V((16, R, 256), F32), V((16, 256, 256), BF),
            V((16, 16, 256), BF), V((8, 256, F), BF), V((8, 2, 256, 256), BF),
            pltpu.SemaphoreType.DMA((18,)), pltpu.SemaphoreType.DMA((8,))],
        compiler_params=pltpu.CompilerParams(vmem_limit_bytes=100 * 1024 * 1024),
    )(A_x.reshape(S // 16, 16, D), A_w_r.T, A_w_i.T, B_w1.T, B_w3.T, B_w2, _FD, _G, _MF)
    return out.reshape(1, S, D)
```
